```python
import jax
import jax.numpy as jnp

def _softmax(x, axis=-1):
    return jax.nn.softmax(x, axis=axis)
def _gelu(x):
    return jax.nn.gelu(x, approximate=True)
def _silu(x):
    return jax.nn.silu(x)
def _sigmoid(x):
    return jax.nn.sigmoid(x)
def _layernorm(x, axis=-1, eps=1e-5):
    m = jnp.mean(x, axis=axis, keepdims=True)
    v = jnp.var(x, axis=axis, keepdims=True)
    return (x - m) / jnp.sqrt(v + eps)
def _scatter_add(tgt, idx, src, axis=0):
    return tgt.at[idx].add(src)
def _segment_sum(src, seg, n):
    return jax.ops.segment_sum(src, seg, n)
class _Rng:
    def __init__(self, key):
        self._k = key
    def _next(self):
        self._k, sub = jax.random.split(self._k)
        return sub
    def normal(self, shape):
        return jax.random.normal(self._next(), shape, dtype=jnp.bfloat16)
    def randint(self, lo, hi, shape):
        return jax.random.randint(self._next(), shape, lo, hi, dtype=jnp.int32)
    def uniform(self, shape, lo=0.0, hi=1.0):
        return jax.random.uniform(self._next(), shape, jnp.bfloat16, lo, hi)
    def permutation(self, n):
        return jax.random.permutation(self._next(), n)


kernel_name = 'recurrent_scan__ssm_conv_h3__mixer_token_mlp__prompt'

def setup_inputs():
    _rng = _Rng(jax.random.key(int.from_bytes(__import__("os").urandom(4), "little")))
    _w = (lambda a: (lambda t: t.astype(jnp.bfloat16) if jnp.issubdtype(t.dtype, jnp.floating) else t)(jnp.asarray(a)))
    def _A_setup():
        B, S, D = 1, 2048, 576
        ks = 4
        return {
            "q": _w((lambda *s: _rng.normal(s) * 0.05)(B, S, D)),
            "k": _w((lambda *s: _rng.normal(s) * 0.05)(B, S, D)),
            "v": _w((lambda *s: _rng.normal(s) * 0.05)(B, S, D)),
            "shift_k": _w((lambda *s: _rng.normal(s) * 0.05)(D, ks) * 0.5),
            "ssm_k": _w((lambda *s: _rng.normal(s) * 0.05)(D, S) * (1.0 / S ** 0.5)),
            "ssm_D": _w((lambda *s: _rng.normal(s) * 0.05)(D)),
        }
    _A_in = _A_setup()

    def _B_setup():
        B, S, D, F = 1, 2048, 576, 4608
        return {
            "x": _w((lambda *s: _rng.normal(s) * 0.05)(B, S, D)),
            "w1": _w((lambda *s: _rng.normal(s) * 0.05)(S, F) * (S ** -0.5)),
            "b1": _w((lambda *s: _rng.normal(s) * 0.05)(F) * 0.02),
            "w2": _w((lambda *s: _rng.normal(s) * 0.05)(F, S) * (F ** -0.5)),
            "b2": _w((lambda *s: _rng.normal(s) * 0.05)(S) * 0.02),
        }
    _B_in = _B_setup()

    return {
        "A_q": _A_in["q"],
        "A_k": _A_in["k"],
        "A_v": _A_in["v"],
        "A_shift_k": _A_in["shift_k"],
        "A_ssm_k": _A_in["ssm_k"],
        "A_ssm_D": _A_in["ssm_D"],
        "B_x": _B_in["x"],
        "B_w1": _B_in["w1"],
        "B_b1": _B_in["b1"],
        "B_w2": _B_in["w2"],
        "B_b2": _B_in["b2"],
    }

def reference(A_q, A_k, A_v, A_shift_k, A_ssm_k, A_ssm_D, B_x, B_w1, B_b1, B_w2, B_b2):
    def _A_ref(q, k, v, shift_k, ssm_k, ssm_D):
        B, S, D = q.shape
        ks = shift_k.shape[-1]
        k_pad = jnp.pad(k, ((0, 0), (ks - 1, 0), (0, 0)))
        k_shift = jnp.zeros_like(k)
        for t in range(ks):
            k_shift = k_shift + k_pad[:, t:t + S, :] * shift_k[:, ks - 1 - t][None, None, :]
        kv = k_shift * v
        L = 2 * S
        kv_pad = jnp.pad(kv, ((0, 0), (0, S), (0, 0)))
        kf_pad = jnp.pad(ssm_k, ((0, 0), (0, S)))
        kv_f = (lambda x, axes=(-2,-1): jnp.fft.rfft2(x.astype(jnp.float32), axes=axes))(kv_pad[:, None, :, :], axes=(1, 2))
        kf_f = (lambda x, axes=(-2,-1): jnp.fft.rfft2(x.astype(jnp.float32), axes=axes))(kf_pad[:, None, :], axes=(1, 2))
        kf_f = (lambda x, *d: x.transpose(*d))(kf_f, 1, 2, 0)
        y_f = kv_f * kf_f[None, :, :, :]
        y = (lambda x, s, axes=(-2,-1): jnp.fft.irfft2(x, s=s, axes=axes).astype(jnp.bfloat16))(y_f, (1, L), axes=(1, 2))[:, 0, :S, :]
        y = y + kv * ssm_D[None, None, :]
        return q * y

    def _B_ref(x, w1, b1, w2, b2):
        B, S, D = x.shape
        h = _layernorm(x, axis=-1)
        u = jnp.einsum("bsd,sf->bdf", h, w1) + b1
        u = _gelu(u)
        y = jnp.einsum("bdf,fs->bds", u, w2) + b2
        return (lambda x, *d: x.transpose(*d))(y, 0, 2, 1)

    x = A_q
    xn = _layernorm(x, axis=-1)
    s = _A_ref(xn, A_k, A_v, A_shift_k, A_ssm_k, A_ssm_D)
    g = _silu(_B_ref(xn, B_w1, B_b1, B_w2, B_b2))
    return x + s * g
```

```python
import functools
import numpy as np
import jax
import jax.numpy as jnp
from jax import lax
from jax.experimental import pallas as pl
from jax.experimental.pallas import tpu as pltpu

S, D, F, KS = 2048, 576, 4608, 4
C = 128
NCH = S // C
TF = 512
N1 = F // TF
TS = 256
N2 = S // TS
EPS = 1e-5
bf16, f32 = jnp.bfloat16, jnp.float32


def _dft_mats():
    t = np.arange(C, dtype=np.float64)[:, None]
    f = np.arange(C, dtype=np.float64)[None, :]
    w = np.exp(-1j * np.pi * (2 * f + 1) * t / (2 * C))
    phi = 1j * (1 - 2 * (np.arange(C) % 2))
    fwd, inv = [], []
    for r in range(4):
        wf = w * phi[None, :] ** (-r)
        fwd.append(np.concatenate([wf.real, wf.imag], axis=1))
        wi = np.conj(w).T * (phi ** r)[:, None] / C
        inv.append(np.concatenate([wi.real, -wi.imag], axis=0))
    return np.stack(fwd).astype(np.float32), np.stack(inv).astype(np.float32)


def _ln_cols(x):
    m = jnp.sum(x, axis=0, keepdims=True) * (1.0 / D)
    d = x - m
    v = jnp.sum(d * d, axis=0, keepdims=True) * (1.0 / D)
    return d * lax.rsqrt(v + EPS)


def _gelu(u):
    return 0.5 * u * (1.0 + jnp.tanh(0.7978845608028654 * (u + 0.044715 * (u * u * u))))


def _build(mb1=(144, 144, 144, 144), zr=16, zg=4, nb=6, cr=48):
    RB = D // nb
    HS = S // 2
    CA = NCH // 2
    NM = len(mb1)

    def kern(sk_hbm, sd_hbm, b1_hbm, b2_hbm, wf_hbm, wi_hbm,
             x_hbm, k_hbm, v_hbm, ssm_hbm, w1_hbm, w2_hbm, o_hbm,
             sk_v, sd_v, b1r_v, b2r_v, wf_v, wi_v,
             x_v, k_v, v_v, ssm_v, w1_v, w2_v, o_v,
             xn_v, h_v, u_v, kv_v, kf_v, xf_v, z_v, b1_v, b2_v, skc_v, dc_v,
             sem_p, sem_x, sem_k, sem_v, sem_s, sem_w1, sem_w2, sem_o):
        acp = pltpu.make_async_copy
        def cx(p): return acp(x_hbm.at[:, pl.ds(p * TS, TS)], x_v.at[p], sem_x.at[p])
        def ck(a): return acp(k_hbm.at[:, pl.ds(a * HS, HS)], k_v.at[:, pl.ds(C + a * HS, HS)], sem_k.at[a])
        def cv(a): return acp(v_hbm.at[:, pl.ds(a * HS, HS)], v_v.at[:, pl.ds(a * HS, HS)], sem_v.at[a])
        def cs(a): return acp(ssm_hbm.at[:, pl.ds(a * HS, HS)], ssm_v.at[:, pl.ds(a * HS, HS)], sem_s.at[a])
        def c1(j): return acp(w1_hbm.at[:, pl.ds(pl.multiple_of(j * TF, TF), TF)], w1_v.at[j], sem_w1.at[j])
        def c2(i): return acp(w2_hbm.at[:, pl.ds(pl.multiple_of(i * TS, TS), TS)], w2_v.at[i], sem_w2.at[i])
        def co(i): return acp(o_v.at[i], o_hbm.at[:, pl.ds(pl.multiple_of(i * TS, TS), TS)], sem_o.at[i])
        small = [acp(s, d_, sem_p.at[n]) for n, (s, d_) in enumerate(
            [(b1_hbm, b1r_v), (b2_hbm, b2r_v), (sk_hbm, sk_v), (sd_hbm, sd_v), (wf_hbm, wf_v), (wi_hbm, wi_v)])]

        for p in range(N2):
            cx(p).start()
        c1(0).start()
        for cp in small:
            cp.start()
        k_v[:, 0:C] = jnp.zeros((D, C), bf16)

        for p in range(N2):
            cx(p).wait()
            if p == 3:
                c1(1).start(); cs(0).start()
            if p == 6:
                ck(0).start(); cv(0).start()
            xn = _ln_cols(x_v[p].astype(f32))
            xn_v[p] = xn
            h_v[:, p * TS:(p + 1) * TS] = _ln_cols(xn).astype(bf16)

        for cp in small:
            cp.wait()
        b1r = b1r_v[...].astype(f32)[None, :]
        for j in range(N1):
            b1_v[j] = b1r[:, j * TF:(j + 1) * TF]
        b2r = b2r_v[...].astype(f32)[None, :]
        for i in range(N2):
            b2_v[i] = b2r[:, i * TS:(i + 1) * TS]
        skr = sk_v[...].astype(f32)
        for t in range(KS):
            skc_v[t] = jnp.broadcast_to(skr[t:t + 1, :], (C, D)).T
        dc_v[...] = jnp.broadcast_to(sd_v[...].astype(f32)[None, :], (C, D)).T

        def mlp1(j, between=None):
            r0 = 0
            for q, mb in enumerate(mb1):
                u = jnp.dot(h_v[r0:r0 + mb, :], w1_v[j], preferred_element_type=f32) + b1_v[j]
                u_v[j, r0:r0 + mb, :] = _gelu(u).astype(bf16)
                r0 += mb
                if between is not None:
                    between(q)

        def issue(n):
            @pl.when(n < N1)
            def _(): c1(n).start()
            @pl.when(jnp.logical_and(n >= N1, n < N1 + N2))
            def _(): c2(n - N1).start()

        c1(2).start()
        cs(1).start(); ck(1).start(); cv(1).start()
        c1(0).wait()
        mlp1(0)

        def shortconv(a, r0, nr):
            kk = k_v[r0:r0 + nr, a * HS:a * HS + C + HS].astype(f32)
            w = [jnp.tile(skc_v[t, r0:r0 + nr, :], (1, CA)) for t in range(KS)]
            ks = kk[:, C:] * w[0]
            for t in range(1, KS):
                ks = ks + kk[:, C - t:C - t + HS] * w[t]
            vv = v_v[r0:r0 + nr, a * HS:(a + 1) * HS].astype(f32)
            kv_v[r0:r0 + nr, a * HS:(a + 1) * HS] = (ks * vv).astype(bf16)

        def fwd_chunk(c):
            kf = jnp.dot(ssm_v[:, c * C:(c + 1) * C], wf_v[c % 4], preferred_element_type=f32)
            if c == 0:
                kf_v[c, :, :C] = kf[:, :C] + dc_v[...]
                kf_v[c, :, C:] = kf[:, C:]
            else:
                kf_v[c] = kf
            xf_v[c] = jnp.dot(kv_v[:, c * C:(c + 1) * C], wf_v[c % 4], preferred_element_type=f32)

        for a in range(2):
            c1(3 + a).start()
            c1(1 + a).wait(); cs(a).wait(); ck(a).wait(); cv(a).wait()

            def between(q, a=a):
                if q == 0:
                    for r0 in range(0, D // 2, cr):
                        shortconv(a, r0, cr)
                elif q == 1:
                    for r0 in range(D // 2, D, cr):
                        shortconv(a, r0, cr)
                elif q == 2:
                    for e in range(CA // 2):
                        fwd_chunk(a * CA + e)
                else:
                    for e in range(CA // 2, CA):
                        fwd_chunk(a * CA + e)
            mlp1(1 + a, between)

        def zblock(r0):
            rows = pl.ds(pl.multiple_of(r0, zr), zr)
            prev = None
            for i0 in range(0, NCH, zg):
                kc, acc = {}, {}
                for j in range(i0 + zg):
                    xr, xi = xf_v[j, rows, :C], xf_v[j, rows, C:]
                    for i in range(max(i0, j), i0 + zg):
                        m = i - j
                        if m not in kc:
                            kc[m] = (kf_v[m, rows, :C], kf_v[m, rows, C:])
                        kr, ki = kc[m]
                        tr = xr * kr - xi * ki
                        ti = xr * ki + xi * kr
                        acc[i] = (tr, ti) if i not in acc else (acc[i][0] + tr, acc[i][1] + ti)
                for i in range(i0, i0 + zg):
                    zr_, zi_ = acc[i]
                    if prev is not None:
                        zr_, zi_ = zr_ + prev[0], zi_ + prev[1]
                    prev = acc[i]
                    z_v[i, rows, :C] = zr_.astype(bf16)
                    z_v[i, rows, C:] = zi_.astype(bf16)

        nsub = RB // zr
        split = [list(range(nsub))[q * nsub // NM:(q + 1) * nsub // NM] for q in range(NM)]

        def b_body(b, _):
            j = 3 + b
            issue(j + 2)
            c1(j).wait()
            mlp1(j, lambda q: [zblock(b * RB + e * zr) for e in split[q]])
            return 0
        lax.fori_loop(0, nb, b_body, 0)

        def p2_body(i, _):
            @pl.when(i + 2 < N2)
            def _(): c2(i + 2).start()
            c2(i).wait()
            y = b2_v[i]
            for j in range(N1):
                y = y + jnp.dot(u_v[j], w2_v[i, j * TF:(j + 1) * TF, :], preferred_element_type=f32)
            g = y * jax.nn.sigmoid(y)
            yc = jnp.concatenate(
                [jnp.dot(z_v[2 * i + e], wi_v[(2 * i + e) % 4], preferred_element_type=f32) for e in range(2)], axis=1)
            o_v[i] = (x_v[i].astype(f32) + xn_v[i] * yc * g).astype(bf16)
            co(i).start()
            return 0
        lax.fori_loop(0, N2, p2_body, 0)
        for i in range(N2):
            co(i).wait()

    hb = pl.BlockSpec(memory_space=pl.ANY)
    V = pltpu.VMEM
    dma = pltpu.SemaphoreType.DMA
    call = pl.pallas_call(
        kern,
        out_shape=jax.ShapeDtypeStruct((D, S), bf16),
        in_specs=[hb] * 12,
        out_specs=hb,
        scratch_shapes=[
            V((KS, D), bf16), V((D,), bf16), V((F,), bf16), V((S,), bf16), V((4, C, 2 * C), bf16), V((4, 2 * C, C), bf16),
            V((N2, D, TS), bf16), V((D, C + S), bf16), V((D, S), bf16), V((D, S), bf16),
            V((N1, S, TF), bf16), V((N2, F, TS), bf16), V((N2, D, TS), bf16),
            V((N2, D, TS), f32), V((D, S), bf16), V((N1, D, TF), bf16), V((D, S), bf16),
            V((NCH, D, 2 * C), f32), V((NCH, D, 2 * C), f32), V((NCH, D, 2 * C), bf16),
            V((N1, 1, TF), f32), V((N2, 1, TS), f32), V((KS, D, C), f32), V((D, C), f32),
            dma((6,)), dma((N2,)), dma((2,)), dma((2,)), dma((2,)), dma((N1,)), dma((N2,)), dma((N2,)),
        ],
        compiler_params=pltpu.CompilerParams(vmem_limit_bytes=120 * 2**20),
    )
    wf, wi = _dft_mats()

    @jax.jit
    def fn(A_q, A_k, A_v, A_shift_k, A_ssm_k, A_ssm_D, B_x, B_w1, B_b1, B_w2, B_b2):
        tr = lambda a: a.reshape(S, D).T
        out = call(A_shift_k.T, A_ssm_D, B_b1, B_b2, jnp.asarray(wf, bf16), jnp.asarray(wi, bf16),
                   tr(A_q), tr(A_k), tr(A_v), A_ssm_k, B_w1, B_w2)
        return out.T.reshape(1, S, D)
    return fn


_FN = _build()


def pallas_recurrent_scan__ssm_conv_h3__mixer_token_mlp__prompt_kernel(
        A_q, A_k, A_v, A_shift_k, A_ssm_k, A_ssm_D, B_x, B_w1, B_b1, B_w2, B_b2):
    return _FN(A_q, A_k, A_v, A_shift_k, A_ssm_k, A_ssm_D, B_x, B_w1, B_b1, B_w2, B_b2)
```

```python
import functools
import numpy as np
import jax
import jax.numpy as jnp
from jax import lax
from jax.experimental import pallas as pl
from jax.experimental.pallas import tpu as pltpu

S, D, F, KS = 2048, 576, 4608, 4
C = 128
NCH = S // C
TF = 512
N1 = F // TF
TS = 256
N2 = S // TS
KG = 512
EPS = 1e-5
bf16, f32, i32, u32 = jnp.bfloat16, jnp.float32, jnp.int32, jnp.uint32
DH = D // 2


def _dft_mats():
    t = np.arange(C, dtype=np.float64)[:, None]
    f = np.arange(C, dtype=np.float64)[None, :]
    w = np.exp(-1j * np.pi * (2 * f + 1) * t / (2 * C))
    phi = 1j * (1 - 2 * (np.arange(C) % 2))
    fwd, inv = [], []
    for r in range(4):
        wf = w * phi[None, :] ** (-r)
        fwd.append(np.concatenate([wf.real, wf.imag], axis=1))
        wi = np.conj(w).T * (phi ** r)[:, None] / C
        inv.append(np.concatenate([wi.real, -wi.imag], axis=0))
    return np.stack(fwd).astype(np.float32), np.stack(inv).astype(np.float32)


def _gelu(u):
    return 0.5 * u * (1.0 + jnp.tanh(0.7978845608028654 * (u + 0.044715 * (u * u * u))))


def pk(x):
    return pltpu.bitcast(x.astype(bf16), u32)


def unpk(x):
    return pltpu.bitcast(x, bf16)


def pin_f32(x, t):
    if t is None:
        return x
    tt = jnp.tile(t, (x.shape[0] // 8, x.shape[1] // 128))
    return pltpu.bitcast(pltpu.bitcast(x, i32) | tt, f32)


def _build(scopes=False, zg=2, zrows=144, nb=4, pin_every=1, wts=(3, 3, 3, 1), flags=None, sc_rows=16):
    ZS = zrows // 16
    import contextlib
    sc = (lambda n: jax.named_scope(n)) if scopes else (lambda n: contextlib.nullcontext())

    def kern(sk_hbm, sd_hbm, b1_hbm, b2_hbm, wf_hbm, wi_hbm,
             x_hbm, k_hbm, v_hbm, ssm_hbm, w1_hbm, w2_hbm, o_hbm,
             sk_v, sd_v, b1r_v, b2r_v, wf_v, wi_v,
             x_v, k_v, v_v, ssm_v, w1_v, w2_v, o_v,
             xn_v, h_v, u_v, kv_v, kf_v, xf_v, z_v, b1_v, b2_v, skc_v, dc_v, y_v, yc_v, zero_v,
             sem_p, sem_w0, sem_x, sem_k, sem_v, sem_s, sem_w1, sem_w2, sem_o):
        acp = pltpu.make_async_copy
        HS = S // 2
        def cx(p): return acp(x_hbm.at[:, pl.ds(p * TS, TS)], x_v.at[p], sem_x.at[p])
        def ck(a): return acp(k_hbm.at[:, pl.ds(a * HS, HS)], k_v.at[a, :, pl.ds(C, HS)], sem_k.at[a])
        def cv(a): return acp(v_hbm.at[:, pl.ds(a * HS, HS)], v_v.at[a], sem_v.at[a])
        ckh = acp(k_hbm.at[:, pl.ds(HS - C, C)], k_v.at[1, :, pl.ds(0, C)], sem_k.at[2])
        def cs(a): return acp(ssm_hbm.at[:, pl.ds(a * HS, HS)], ssm_v.at[:, pl.ds(a * HS, HS)], sem_s.at[a])
        def c1(j): return acp(w1_hbm.at[:, pl.ds(pl.multiple_of(j * TF, TF), TF)], w1_v.at[j], sem_w1.at[j])
        def c2(i): return acp(w2_hbm.at[:, pl.ds(pl.multiple_of(i * TS, TS), TS)], w2_v.at[i], sem_w2.at[i])
        def co(c): return acp(o_v.at[c], o_hbm.at[:, pl.ds(pl.multiple_of(c * C, C), C)], sem_o.at[c])
        small = [acp(s, d_, sem_p.at[n]) for n, (s, d_) in enumerate(
            [(b1_hbm, b1r_v), (b2_hbm, b2r_v), (sk_hbm, sk_v), (sd_hbm, sd_v), (wf_hbm, wf_v), (wi_hbm, wi_v)])]

        def c1p(kg): return acp(w1_hbm.at[pl.ds(kg * KG, KG), pl.ds(0, TF)], w1_v.at[0, pl.ds(kg * KG, KG), :], sem_w0.at[kg])
        cx(0).start(); cx(1).start(); c1p(0).start()
        cx(2).start(); cx(3).start(); c1p(1).start()
        small[0].start()
        zero_v[...] = jnp.zeros((8, C), i32)

        def ln_steps(p):
            A, B, Cc = [], [], []
            for e in range(TS // C):
                ls = slice(e * C, (e + 1) * C)
                st_ = {}
                nrb = D // 16
                for rb in range(nrb):
                    rs = slice(16 * rb, 16 * rb + 16)
                    def sa(pin, rs=rs, rb=rb, ls=ls, st_=st_):
                        xf = pin_f32(x_v[p, rs, ls].astype(f32), None if pin is None else pin())
                        st_["a"] = xf if rb == 0 else st_["a"] + xf
                        if rb == nrb - 1:
                            st_["m"] = jnp.sum(st_["a"], axis=0, keepdims=True) * (1.0 / D)
                    def sb(pin, rs=rs, rb=rb, ls=ls, st_=st_):
                        d = pin_f32(x_v[p, rs, ls].astype(f32), None if pin is None else pin()) - st_["m"]
                        xn_v[p, rs, ls] = d
                        st_["s1"] = d if rb == 0 else st_["s1"] + d
                        st_["s2"] = d * d if rb == 0 else st_["s2"] + d * d
                        if rb == nrb - 1:
                            e_ = jnp.sum(st_["s1"], axis=0, keepdims=True) * (1.0 / D)
                            v = jnp.sum(st_["s2"], axis=0, keepdims=True) * (1.0 / D)
                            r = lax.rsqrt(v + EPS)
                            r2 = lax.rsqrt(r * r * (v - e_ * e_) + EPS)
                            st_["e"], st_["r"], st_["rr"] = e_, r, r * r2
                    def sc_(pin, rs=rs, rb=rb, ls=ls, e=e, st_=st_):
                        d = pin_f32(xn_v[p, rs, ls], None if pin is None else pin())
                        xn_v[p, rs, ls] = d * st_["r"]
                        h_v[8 * rb:8 * rb + 8, p * TS + e * C:p * TS + (e + 1) * C] = pk((d - st_["e"]) * st_["rr"])
                    A.append(sa); B.append(sb); Cc.append(sc_)
            mix = lambda L: [x for pair in zip(L[:len(L) // 2], L[len(L) // 2:]) for x in pair]
            return mix(A), mix(B), mix(Cc)

        def prep_steps():
            out = []
            def fill(pin):
                k_v[0, :, 0:C] = jnp.zeros((D, C), bf16)
                y_v[1] = jnp.zeros((D, C), f32)
                yc_v[1] = jnp.zeros((D, C), f32)
                b2r = b2r_v[...].astype(f32)[None, :]
                for i in range(N2):
                    b2_v[i] = b2r[:, i * TS:(i + 1) * TS]
            out.append(fill)
            for t in range(KS + 1):
                for c0 in range(0, D, C):
                    w = min(C, D - c0)
                    def st(pin, t=t, c0=c0, w=w):
                        row = sk_v[t:t + 1, c0:c0 + w].astype(f32) if t < KS else sd_v[...].astype(f32)[None, c0:c0 + w]
                        tile = jnp.broadcast_to(row, (C, w))
                        if w == C:
                            tile = pin_f32(tile, pin())
                        if t < KS:
                            skc_v[t, c0:c0 + w, :] = tile.T
                        else:
                            dc_v[c0:c0 + w, :] = tile.T
                    out.append(st)
            return out

        for p in range(2):
            with sc('p0w%d' % p):
                cx(p).wait()
            with sc('p0c%d' % p):
                for L in ln_steps(p):
                    for st in L:
                        st(None)

        def run_pinned(y, steps):
            n = len(steps)
            z0 = zero_v[...]
            nv = y.shape[0] // 8
            for q, st in enumerate(steps):
                s = min(nv - 1, (q * nv) // n)
                st(lambda s=s: pltpu.bitcast(y[8 * s:8 * s + 8, 0:C], i32) & z0)

        def share(steps, weights):
            tot = sum(weights); out = []; lo = 0; acc = 0
            for w in weights:
                acc += w
                hi = (len(steps) * acc) // tot
                out.append(steps[lo:hi]); lo = hi
            return out

        def mlp1(j, steps=(), seg_w=None, after=None):
            segs = [(n, kg) for n in range(TF // C) for kg in range(S // KG)]
            w = seg_w if seg_w is not None else [wts[kg] for (n, kg) in segs]
            sh = share(list(steps), w)
            acc = None
            for q, (n, kg) in enumerate(segs):
                lhs = unpk(h_v[:, kg * KG:(kg + 1) * KG])
                y = jnp.dot(lhs, w1_v[j, kg * KG:(kg + 1) * KG, n * C:(n + 1) * C], preferred_element_type=f32)
                acc = y + b1_v[j, :, n * C:(n + 1) * C] if kg == 0 else acc + y
                if kg == S // KG - 1:
                    u_v[j, :, n * C:(n + 1) * C] = pk(_gelu(acc))
                run_pinned(y, sh[q])
                if after is not None:
                    after(q)

        with sc('s0'):
            accs = [None] * 4
            for kg in range(4):
                if kg + 2 < 4:
                    cx(2 * kg + 4).start(); cx(2 * kg + 5).start(); c1p(kg + 2).start()
                elif kg == 2:
                    c1(1).start()
                else:
                    for cp in small[1:]:
                        cp.start()
                if kg < 3:
                    cx(2 * kg + 2).wait(); cx(2 * kg + 3).wait()
                    A0, B0, C0 = ln_steps(2 * kg + 2)
                    A1, B1, C1 = ln_steps(2 * kg + 3)
                    zz = lambda a, b: [x for pair in zip(a, b) for x in pair]
                    work = [zz(A0, A1), zz(B0, B1), zz(C0, C1), []]
                else:
                    work = [[], [], [], []]
                c1p(kg).wait()
                if kg == 3:
                    small[0].wait()
                    b1r = b1r_v[...].astype(f32)[None, :]
                    for j in range(N1):
                        b1_v[j] = b1r[:, j * TF:(j + 1) * TF]
                for n in range(4):
                    y = jnp.dot(unpk(h_v[:, kg * KG:(kg + 1) * KG]), w1_v[0, kg * KG:(kg + 1) * KG, n * C:(n + 1) * C],
                                preferred_element_type=f32)
                    accs[n] = y if kg == 0 else accs[n] + y
                    if kg == 3:
                        u_v[0, :, n * C:(n + 1) * C] = pk(_gelu(accs[n] + b1_v[0, :, n * C:(n + 1) * C]))
                    run_pinned(y, work[n])

        def sc_steps(a):
            out = []
            for r0 in range(0, D, sc_rows):
                def st(pin, r0=r0):
                    rs = slice(r0, r0 + sc_rows)
                    kk = pin_f32(k_v[a, rs, :].astype(f32), pin())
                    ks = kk[:, C:] * jnp.tile(skc_v[0, rs, :], (1, HS // C))
                    for t in range(1, KS):
                        ks = ks + kk[:, C - t:C - t + HS] * jnp.tile(skc_v[t, rs, :], (1, HS // C))
                    vv = v_v[a, rs, :].astype(f32)
                    kv_v[a, r0 // 2:(r0 + sc_rows) // 2, :] = pk(ks * vv)
                out.append(st)
            return out

        def xdft(a, e):
            xf_v[a * 8 + e] = jnp.dot(unpk(kv_v[a, :, e * C:(e + 1) * C]), wf_v[e % 4], preferred_element_type=f32)

        def kdft(c):
            kf = jnp.dot(ssm_v[:, c * C:(c + 1) * C], wf_v[c % 4], preferred_element_type=f32)
            if c == 0:
                kf_v[c, :, :C] = kf[:, :C] + dc_v[...]
                kf_v[c, :, C:] = kf[:, C:]
            else:
                kf_v[c] = kf

        c1(2).start(); ck(0).start(); ckh.start(); cv(0).start()
        with sc('w1'):
            c1(1).wait()
            for cp in small[1:]:
                cp.wait()
        with sc('s1'):
            mlp1(1, prep_steps(), seg_w=[1] * 16)

        def a_body(a, _):
            j = 2 + a
            @pl.when(a == 0)
            def _(): c1(3).start(); ck(1).start(); cv(1).start()
            @pl.when(a == 1)
            def _(): c1(4).start(); cs(0).start(); cs(1).start()
            with sc('wA'):
                c1(j).wait(); ck(a).wait(); cv(a).wait()
            with sc('sA'):
                mlp1(j, sc_steps(a), seg_w=[1] * 8 + [0] * 8,
                     after=lambda q: xdft(a, q - 8) if q >= 8 else None)
            return 0
        ckh.wait()
        lax.fori_loop(0, 2, a_body, 0)

        c1(5).start()
        with sc('w4'):
            c1(4).wait(); cs(0).wait(); cs(1).wait()
        with sc('sK'):
            mlp1(4, after=lambda q: kdft(q))

        def z_steps(r0):
            rows = pl.ds(pl.multiple_of(r0, 16), 16)
            rowsh = pl.ds(pl.multiple_of(r0 // 2, 8), 8)
            st_ = {"prev": None}
            out = []
            for i0 in range(0, NCH, zg):
                kc, acc = {}, {}
                for j in range(i0 + zg):
                    def st(pin, i0=i0, j=j, kc=kc, acc=acc):
                        xr, xi = xf_v[j, rows, :C], xf_v[j, rows, C:]
                        if j % pin_every == 0:
                            xr = pin_f32(xr, pin())
                        for i in range(max(i0, j), i0 + zg):
                            m = i - j
                            if m not in kc:
                                kc[m] = (kf_v[m, rows, :C], kf_v[m, rows, C:])
                            kr, ki = kc[m]
                            tr = xr * kr - xi * ki
                            ti = xr * ki + xi * kr
                            acc[i] = (tr, ti) if i not in acc else (acc[i][0] + tr, acc[i][1] + ti)
                        if j == i0 + zg - 1:
                            for i in range(i0, i0 + zg):
                                zr_, zi_ = acc[i]
                                if st_["prev"] is not None:
                                    zr_, zi_ = zr_ + st_["prev"][0], zi_ + st_["prev"][1]
                                st_["prev"] = acc[i]
                                z_v[i, rowsh, :C] = pk(zr_)
                                z_v[i, rowsh, C:] = pk(zi_)
                    out.append(st)
            return out

        def b_body(b, _):
            j = 5 + b
            @pl.when(j + 1 < N1)
            def _(): c1(j + 1).start()
            @pl.when(j >= N1 - 2)
            def _(): c2(j - (N1 - 2)).start()
            with sc('wb'):
                c1(j).wait()
            r0 = jnp.minimum(b * zrows, D - zrows)
            steps = []
            for e in range(ZS):
                steps += z_steps(r0 + e * 16)
            with sc('sb'):
                mlp1(j, steps)
            return 0
        lax.fori_loop(0, nb, b_body, 0)

        def ep_steps(slot, p, e, c):
            out = []
            for r0 in range(0, D, 16):
                def st(pin, r0=r0):
                    rs = slice(r0, r0 + 16)
                    y = pin_f32(y_v[slot, rs, :], None if pin is None else pin())
                    g = y * jax.nn.sigmoid(y)
                    o = x_v[p, rs, e * C:(e + 1) * C].astype(f32) + xn_v[p, rs, e * C:(e + 1) * C] * yc_v[slot, rs, :] * g
                    o_v[c, rs, :] = o.astype(bf16)
                out.append(st)
            return out

        def mlp2_chunk(i, e, steps, slot):
            sh = share(steps, [1] * N1)
            acc = None
            for kg in range(N1):
                y = jnp.dot(unpk(u_v[kg]), w2_v[i, kg * KG:(kg + 1) * KG, e * C:(e + 1) * C], preferred_element_type=f32)
                acc = y + b2_v[i, :, e * C:(e + 1) * C] if kg == 0 else acc + y
                run_pinned(y, sh[kg])
                if kg == 1:
                    c = 2 * i + e
                    yc_v[slot] = jnp.dot(unpk(z_v[c]), wi_v[c % 4], preferred_element_type=f32)
            y_v[slot] = acc

        def p2_body(i, _):
            @pl.when(i + 2 < N2)
            def _(): c2(i + 2).start()
            with sc('w2'):
                c2(i).wait()
            ip = jnp.maximum(i - 1, 0)
            prev_slot = jnp.where(i == 0, 1, 3)
            prev_c = jnp.where(i == 0, NCH, 2 * i - 1)
            with sc('p2a'):
                mlp2_chunk(i, 0, ep_steps(prev_slot, ip, 1, prev_c), 2)
            @pl.when(i > 0)
            def _(): co(2 * i - 1).start()
            with sc('p2b'):
                mlp2_chunk(i, 1, ep_steps(2, i, 0, 2 * i), 3)
            co(2 * i).start()
            return 0
        lax.fori_loop(0, N2, p2_body, 0)
        for st in ep_steps(3, N2 - 1, 1, NCH - 1):
            st(None)
        co(NCH - 1).start()
        with sc('tailwait'):
            for c in range(NCH):
                co(c).wait()

    hb = pl.BlockSpec(memory_space=pl.ANY)
    V = pltpu.VMEM
    dma = pltpu.SemaphoreType.DMA
    call = pl.pallas_call(
        kern,
        out_shape=jax.ShapeDtypeStruct((D, S), bf16),
        in_specs=[hb] * 12,
        out_specs=hb,
        scratch_shapes=[
            V((KS, D), bf16), V((D,), bf16), V((F,), bf16), V((S,), bf16), V((4, C, 2 * C), bf16), V((4, 2 * C, C), bf16),
            V((N2, D, TS), bf16), V((2, D, C + S // 2), bf16), V((2, D, S // 2), bf16), V((D, S), bf16),
            V((N1, S, TF), bf16), V((N2, F, TS), bf16), V((NCH + 1, D, C), bf16),
            V((N2, D, TS), f32), V((DH, S), u32), V((N1, DH, TF), u32), V((2, DH, S // 2), u32),
            V((NCH, D, 2 * C), f32), V((NCH, D, 2 * C), f32), V((NCH, DH, 2 * C), u32),
            V((N1, 1, TF), f32), V((N2, 1, TS), f32), V((KS, D, C), f32), V((D, C), f32),
            V((4, D, C), f32), V((4, D, C), f32), V((8, C), i32),
            dma((6,)), dma((4,)), dma((N2,)), dma((3,)), dma((2,)), dma((2,)), dma((N1,)), dma((N2,)), dma((NCH,)),
        ],
        compiler_params=pltpu.CompilerParams(vmem_limit_bytes=120 * 2**20, flags=flags),
    )
    wf, wi = _dft_mats()

    @jax.jit
    def fn(A_q, A_k, A_v, A_shift_k, A_ssm_k, A_ssm_D, B_x, B_w1, B_b1, B_w2, B_b2):
        tr = lambda a: a.reshape(S, D).T
        out = call(A_shift_k.T, A_ssm_D, B_b1, B_b2, jnp.asarray(wf, bf16), jnp.asarray(wi, bf16),
                   tr(A_q), tr(A_k), tr(A_v), A_ssm_k, B_w1, B_w2)
        return out.T.reshape(1, S, D)
    return fn


_FN = _build()


def pallas_recurrent_scan__ssm_conv_h3__mixer_token_mlp__prompt_kernel(
        A_q, A_k, A_v, A_shift_k, A_ssm_k, A_ssm_D, B_x, B_w1, B_b1, B_w2, B_b2):
    return _FN(A_q, A_k, A_v, A_shift_k, A_ssm_k, A_ssm_D, B_x, B_w1, B_b1, B_w2, B_b2)
```

```python
import functools
import numpy as np
import jax
import jax.numpy as jnp
from jax import lax
from jax.experimental import pallas as pl
from jax.experimental.pallas import tpu as pltpu

S, D, F, KS = 2048, 576, 4608, 4
C = 128
NCH = S // C
TF = 512
N1 = F // TF
TS = 256
N2 = S // TS
KG = 512
EPS = 1e-5
bf16, f32, i32, u32 = jnp.bfloat16, jnp.float32, jnp.int32, jnp.uint32
DH = D // 2


def _dft_mats():
    t = np.arange(C, dtype=np.float64)[:, None]
    f = np.arange(C, dtype=np.float64)[None, :]
    w = np.exp(-1j * np.pi * (2 * f + 1) * t / (2 * C))
    phi = 1j * (1 - 2 * (np.arange(C) % 2))
    fwd, inv = [], []
    for r in range(4):
        wf = w * phi[None, :] ** (-r)
        fwd.append(np.concatenate([wf.real, wf.imag], axis=1))
        wi = np.conj(w).T * (phi ** r)[:, None] / C
        inv.append(np.concatenate([wi.real, -wi.imag], axis=0))
    return np.stack(fwd).astype(np.float32), np.stack(inv).astype(np.float32)


def _gelu(u):
    return 0.5 * u * (1.0 + jnp.tanh(0.7978845608028654 * (u + 0.044715 * (u * u * u))))


def pk(x):
    return pltpu.bitcast(x.astype(bf16), u32)


def unpk(x):
    return pltpu.bitcast(x, bf16)


def pin_f32(x, t):
    if t is None:
        return x
    tt = jnp.tile(t, (x.shape[0] // 8, x.shape[1] // 128))
    return pltpu.bitcast(pltpu.bitcast(x, i32) | tt, f32)


def _build(scopes=False, zg=2, zrows=144, nb=4, pin_every=1, wts=(3, 3, 3, 1), flags=None, sc_rows=16):
    ZS = zrows // 16
    import contextlib
    sc = lambda n: jax.named_scope(n) if (scopes and (scopes == 2 or n.startswith('w') or n.startswith('p0w') or n.startswith('tail'))) else contextlib.nullcontext()

    def kern(sk_hbm, sd_hbm, b1_hbm, b2_hbm, wf_hbm, wi_hbm,
             x_hbm, k_hbm, v_hbm, ssm_hbm, w1_hbm, w2_hbm, o_hbm,
             sk_v, sd_v, b1r_v, b2r_v, wf_v, wi_v,
             x_v, k_v, v_v, ssm_v, w1_v, w2_v, o_v,
             xn_v, h_v, u_v, kv_v, kf_v, xf_v, z_v, b1_v, b2_v, skc_v, dc_v, y_v, yc_v, zero_v,
             sem_p, sem_w0, sem_x, sem_kv, sem_w1, sem_w2, sem_o):
        acp = pltpu.make_async_copy
        HS = S // 2
        def cx(p): return acp(x_hbm.at[:, pl.ds(p * TS, TS)], x_v.at[p], sem_x.at[p % 4])
        def ck(a): return acp(k_hbm.at[:, pl.ds(a * HS, HS)], k_v.at[a, :, pl.ds(C, HS)], sem_kv.at[a])
        def cv(a): return acp(v_hbm.at[:, pl.ds(a * HS, HS)], v_v.at[a], sem_kv.at[a])
        ckh = acp(k_hbm.at[:, pl.ds(HS - C, C)], k_v.at[1, :, pl.ds(0, C)], sem_kv.at[1])
        def cs(a): return acp(ssm_hbm.at[:, pl.ds(a * HS, HS)], ssm_v.at[:, pl.ds(a * HS, HS)], sem_p.at[2])
        def c1(j): return acp(w1_hbm.at[:, pl.ds(pl.multiple_of(j * TF, TF), TF)], w1_v.at[j], sem_w1.at[j % 2])
        def c2(i): return acp(w2_hbm.at[:, pl.ds(pl.multiple_of(i * TS, TS), TS)], w2_v.at[i], sem_w2.at[i % 3])
        def co(c): return acp(o_v.at[c], o_hbm.at[:, pl.ds(pl.multiple_of(c * C, C), C)], sem_o.at[0])
        small = [acp(s, d_, sem_p.at[min(n, 1)]) for n, (s, d_) in enumerate(
            [(b1_hbm, b1r_v), (b2_hbm, b2r_v), (sk_hbm, sk_v), (sd_hbm, sd_v), (wf_hbm, wf_v), (wi_hbm, wi_v)])]

        def c1p(kg): return acp(w1_hbm.at[pl.ds(kg * KG, KG), pl.ds(0, TF)], w1_v.at[0, pl.ds(kg * KG, KG), :], sem_w0.at[kg % 2])
        cx(0).start(); cx(1).start(); c1p(0).start()
        cx(2).start(); cx(3).start(); c1p(1).start()
        small[0].start()
        zero_v[...] = jnp.zeros((8, C), i32)

        def ln_steps(p):
            A, B, Cc = [], [], []
            for e in range(TS // C):
                ls = slice(e * C, (e + 1) * C)
                st_ = {}
                nrb = D // 16
                for rb in range(nrb):
                    rs = slice(16 * rb, 16 * rb + 16)
                    def sa(pin, rs=rs, rb=rb, ls=ls, st_=st_):
                        xf = pin_f32(x_v[p, rs, ls].astype(f32), None if pin is None else pin())
                        st_["a"] = xf if rb == 0 else st_["a"] + xf
                        if rb == nrb - 1:
                            st_["m"] = jnp.sum(st_["a"], axis=0, keepdims=True) * (1.0 / D)
                    def sb(pin, rs=rs, rb=rb, ls=ls, st_=st_):
                        d = pin_f32(x_v[p, rs, ls].astype(f32), None if pin is None else pin()) - st_["m"]
                        xn_v[p, rs, ls] = d
                        st_["s1"] = d if rb == 0 else st_["s1"] + d
                        st_["s2"] = d * d if rb == 0 else st_["s2"] + d * d
                        if rb == nrb - 1:
                            e_ = jnp.sum(st_["s1"], axis=0, keepdims=True) * (1.0 / D)
                            v = jnp.sum(st_["s2"], axis=0, keepdims=True) * (1.0 / D)
                            r = lax.rsqrt(v + EPS)
                            r2 = lax.rsqrt(r * r * (v - e_ * e_) + EPS)
                            st_["e"], st_["r"], st_["rr"] = e_, r, r * r2
                    def sc_(pin, rs=rs, rb=rb, ls=ls, e=e, st_=st_):
                        d = pin_f32(xn_v[p, rs, ls], None if pin is None else pin())
                        xn_v[p, rs, ls] = d * st_["r"]
                        h_v[8 * rb:8 * rb + 8, p * TS + e * C:p * TS + (e + 1) * C] = pk((d - st_["e"]) * st_["rr"])
                    A.append(sa); B.append(sb); Cc.append(sc_)
            mix = lambda L: [x for pair in zip(L[:len(L) // 2], L[len(L) // 2:]) for x in pair]
            return mix(A), mix(B), mix(Cc)

        def prep_steps():
            out = []
            def fill(pin):
                k_v[0, :, 0:C] = jnp.zeros((D, C), bf16)
                y_v[1] = jnp.zeros((D, C), f32)
                yc_v[1] = jnp.zeros((D, C), f32)
                b2r = b2r_v[...].astype(f32)[None, :]
                for i in range(N2):
                    b2_v[i] = b2r[:, i * TS:(i + 1) * TS]
            out.append(fill)
            for t in range(KS + 1):
                for c0 in range(0, D, C):
                    w = min(C, D - c0)
                    def st(pin, t=t, c0=c0, w=w):
                        row = sk_v[t:t + 1, c0:c0 + w].astype(f32) if t < KS else sd_v[...].astype(f32)[None, c0:c0 + w]
                        tile = jnp.broadcast_to(row, (C, w))
                        if w == C:
                            tile = pin_f32(tile, pin())
                        if t < KS:
                            skc_v[t, c0:c0 + w, :] = tile.T
                        else:
                            dc_v[c0:c0 + w, :] = tile.T
                    out.append(st)
            return out

        for p in range(2):
            with sc('p0w%d' % p):
                cx(p).wait()
            with sc('p0c%d' % p):
                for L in ln_steps(p):
                    for st in L:
                        st(None)

        def run_pinned(y, steps):
            n = len(steps)
            z0 = zero_v[...]
            nv = y.shape[0] // 8
            for q, st in enumerate(steps):
                s = min(nv - 1, (q * nv) // n)
                st(lambda s=s: pltpu.bitcast(y[8 * s:8 * s + 8, 0:C], i32) & z0)

        def share(steps, weights):
            tot = sum(weights); out = []; lo = 0; acc = 0
            for w in weights:
                acc += w
                hi = (len(steps) * acc) // tot
                out.append(steps[lo:hi]); lo = hi
            return out

        def mlp1(j, steps=(), seg_w=None, after=None):
            segs = [(n, kg) for n in range(TF // C) for kg in range(S // KG)]
            w = seg_w if seg_w is not None else [wts[kg] for (n, kg) in segs]
            sh = share(list(steps), w)
            acc = None
            for q, (n, kg) in enumerate(segs):
                lhs = unpk(h_v[:, kg * KG:(kg + 1) * KG])
                y = jnp.dot(lhs, w1_v[j, kg * KG:(kg + 1) * KG, n * C:(n + 1) * C], preferred_element_type=f32)
                acc = y + b1_v[j, :, n * C:(n + 1) * C] if kg == 0 else acc + y
                if kg == S // KG - 1:
                    u_v[j, :, n * C:(n + 1) * C] = pk(_gelu(acc))
                run_pinned(y, sh[q])
                if after is not None:
                    after(q)

        with sc('s0'):
            accs = [None] * 4
            for kg in range(4):
                if kg + 2 < 4:
                    cx(2 * kg + 4).start(); cx(2 * kg + 5).start()
                elif kg == 2:
                    c1(1).start()
                else:
                    for cp in small[1:]:
                        cp.start()
                if kg < 3:
                    cx(2 * kg + 2).wait(); cx(2 * kg + 3).wait()
                    A0, B0, C0 = ln_steps(2 * kg + 2)
                    A1, B1, C1 = ln_steps(2 * kg + 3)
                    zz = lambda a, b: [x for pair in zip(a, b) for x in pair]
                    work = [zz(A0, A1), zz(B0, B1), zz(C0, C1), []]
                else:
                    work = [[], [], [], []]
                c1p(kg).wait()
                if kg + 2 < 4:
                    c1p(kg + 2).start()
                if kg == 3:
                    small[0].wait()
                    b1r = b1r_v[...].astype(f32)[None, :]
                    for j in range(N1):
                        b1_v[j] = b1r[:, j * TF:(j + 1) * TF]
                for n in range(4):
                    y = jnp.dot(unpk(h_v[:, kg * KG:(kg + 1) * KG]), w1_v[0, kg * KG:(kg + 1) * KG, n * C:(n + 1) * C],
                                preferred_element_type=f32)
                    accs[n] = y if kg == 0 else accs[n] + y
                    if kg == 3:
                        u_v[0, :, n * C:(n + 1) * C] = pk(_gelu(accs[n] + b1_v[0, :, n * C:(n + 1) * C]))
                    run_pinned(y, work[n])

        def sc_steps(a):
            out = []
            for r0 in range(0, D, sc_rows):
                def st(pin, r0=r0):
                    rs = slice(r0, r0 + sc_rows)
                    kk = pin_f32(k_v[a, rs, :].astype(f32), pin())
                    ks = kk[:, C:] * jnp.tile(skc_v[0, rs, :], (1, HS // C))
                    for t in range(1, KS):
                        ks = ks + kk[:, C - t:C - t + HS] * jnp.tile(skc_v[t, rs, :], (1, HS // C))
                    vv = v_v[a, rs, :].astype(f32)
                    kv_v[a, r0 // 2:(r0 + sc_rows) // 2, :] = pk(ks * vv)
                out.append(st)
            return out

        def xdft(a, e):
            xf_v[a * 8 + e] = jnp.dot(unpk(kv_v[a, :, e * C:(e + 1) * C]), wf_v[e % 4], preferred_element_type=f32)

        def kdft(c):
            kf = jnp.dot(ssm_v[:, c * C:(c + 1) * C], wf_v[c % 4], preferred_element_type=f32)
            if c == 0:
                kf_v[c, :, :C] = kf[:, :C] + dc_v[...]
                kf_v[c, :, C:] = kf[:, C:]
            else:
                kf_v[c] = kf

        c1(2).start(); ck(0).start(); cv(0).start()
        with sc('w1'):
            c1(1).wait()
            for cp in small[1:]:
                cp.wait()
        with sc('s1'):
            mlp1(1, prep_steps(), seg_w=[1] * 16)

        def a_body(a, _):
            j = 2 + a
            @pl.when(a == 0)
            def _(): c1(3).start(); ck(1).start(); cv(1).start(); ckh.start()
            @pl.when(a == 1)
            def _(): c1(4).start(); cs(0).start(); cs(1).start()
            with sc('wA'):
                c1(j).wait(); ck(a).wait(); cv(a).wait()
                @pl.when(a == 1)
                def _(): ckh.wait()
            with sc('sA'):
                mlp1(j, sc_steps(a), seg_w=[1] * 8 + [0] * 8,
                     after=lambda q: xdft(a, q - 8) if q >= 8 else None)
            return 0
        lax.fori_loop(0, 2, a_body, 0)

        c1(5).start()
        with sc('w4'):
            c1(4).wait(); cs(0).wait(); cs(1).wait()
        with sc('sK'):
            mlp1(4, after=lambda q: kdft(q))

        def z_steps(r0):
            rows = pl.ds(pl.multiple_of(r0, 16), 16)
            rowsh = pl.ds(pl.multiple_of(r0 // 2, 8), 8)
            st_ = {"prev": None}
            out = []
            for i0 in range(0, NCH, zg):
                kc, acc = {}, {}
                for j in range(i0 + zg):
                    def st(pin, i0=i0, j=j, kc=kc, acc=acc):
                        xr, xi = xf_v[j, rows, :C], xf_v[j, rows, C:]
                        if j % pin_every == 0:
                            xr = pin_f32(xr, pin())
                        for i in range(max(i0, j), i0 + zg):
                            m = i - j
                            if m not in kc:
                                kc[m] = (kf_v[m, rows, :C], kf_v[m, rows, C:])
                            kr, ki = kc[m]
                            tr = xr * kr - xi * ki
                            ti = xr * ki + xi * kr
                            acc[i] = (tr, ti) if i not in acc else (acc[i][0] + tr, acc[i][1] + ti)
                        if j == i0 + zg - 1:
                            for i in range(i0, i0 + zg):
                                zr_, zi_ = acc[i]
                                if st_["prev"] is not None:
                                    zr_, zi_ = zr_ + st_["prev"][0], zi_ + st_["prev"][1]
                                st_["prev"] = acc[i]
                                z_v[i, rowsh, :C] = pk(zr_)
                                z_v[i, rowsh, C:] = pk(zi_)
                    out.append(st)
            return out

        def b_body(b, _):
            j = 5 + b
            @pl.when(j + 1 < N1)
            def _(): c1(j + 1).start()
            @pl.when(j >= N1 - 2)
            def _(): c2(j - (N1 - 2)).start()
            with sc('wb'):
                c1(j).wait()
            r0 = jnp.minimum(b * zrows, D - zrows)
            steps = []
            for e in range(ZS):
                steps += z_steps(r0 + e * 16)
            with sc('sb'):
                mlp1(j, steps)
            return 0
        lax.fori_loop(0, nb, b_body, 0)

        def ep_steps(slot, p, e, c):
            out = []
            for r0 in range(0, D, 16):
                def st(pin, r0=r0):
                    rs = slice(r0, r0 + 16)
                    y = pin_f32(y_v[slot, rs, :], None if pin is None else pin())
                    g = y * jax.nn.sigmoid(y)
                    o = x_v[p, rs, e * C:(e + 1) * C].astype(f32) + xn_v[p, rs, e * C:(e + 1) * C] * yc_v[slot, rs, :] * g
                    o_v[c, rs, :] = o.astype(bf16)
                out.append(st)
            return out

        def mlp2_chunk(i, e, steps, slot):
            sh = share(steps, [1] * N1)
            acc = None
            for kg in range(N1):
                y = jnp.dot(unpk(u_v[kg]), w2_v[i, kg * KG:(kg + 1) * KG, e * C:(e + 1) * C], preferred_element_type=f32)
                acc = y + b2_v[i, :, e * C:(e + 1) * C] if kg == 0 else acc + y
                run_pinned(y, sh[kg])
                if kg == 1:
                    c = 2 * i + e
                    yc_v[slot] = jnp.dot(unpk(z_v[c]), wi_v[c % 4], preferred_element_type=f32)
            y_v[slot] = acc

        def p2_body(i, _):
            @pl.when(i + 2 < N2)
            def _(): c2(i + 2).start()
            with sc('w2'):
                c2(i).wait()
            ip = jnp.maximum(i - 1, 0)
            prev_slot = jnp.where(i == 0, 1, 3)
            prev_c = jnp.where(i == 0, NCH, 2 * i - 1)
            with sc('p2a'):
                mlp2_chunk(i, 0, ep_steps(prev_slot, ip, 1, prev_c), 2)
            @pl.when(i > 0)
            def _(): co(2 * i - 1).start()
            with sc('p2b'):
                mlp2_chunk(i, 1, ep_steps(2, i, 0, 2 * i), 3)
            co(2 * i).start()
            return 0
        lax.fori_loop(0, N2, p2_body, 0)
        for st in ep_steps(3, N2 - 1, 1, NCH - 1):
            st(None)
        co(NCH - 1).start()
        with sc('tailwait'):
            for c in range(NCH):
                co(c).wait()

    hb = pl.BlockSpec(memory_space=pl.ANY)
    V = pltpu.VMEM
    dma = pltpu.SemaphoreType.DMA
    call = pl.pallas_call(
        kern,
        out_shape=jax.ShapeDtypeStruct((D, S), bf16),
        in_specs=[hb] * 12,
        out_specs=hb,
        scratch_shapes=[
            V((KS, D), bf16), V((D,), bf16), V((F,), bf16), V((S,), bf16), V((4, C, 2 * C), bf16), V((4, 2 * C, C), bf16),
            V((N2, D, TS), bf16), V((2, D, C + S // 2), bf16), V((2, D, S // 2), bf16), V((D, S), bf16),
            V((N1, S, TF), bf16), V((N2, F, TS), bf16), V((NCH + 1, D, C), bf16),
            V((N2, D, TS), f32), V((DH, S), u32), V((N1, DH, TF), u32), V((2, DH, S // 2), u32),
            V((NCH, D, 2 * C), f32), V((NCH, D, 2 * C), f32), V((NCH, DH, 2 * C), u32),
            V((N1, 1, TF), f32), V((N2, 1, TS), f32), V((KS, D, C), f32), V((D, C), f32),
            V((4, D, C), f32), V((4, D, C), f32), V((8, C), i32),
            dma((3,)), dma((2,)), dma((4,)), dma((2,)), dma((2,)), dma((3,)), dma((1,)),
        ],
        compiler_params=pltpu.CompilerParams(vmem_limit_bytes=120 * 2**20, flags=flags),
    )
    wf, wi = _dft_mats()

    @jax.jit
    def fn(A_q, A_k, A_v, A_shift_k, A_ssm_k, A_ssm_D, B_x, B_w1, B_b1, B_w2, B_b2):
        tr = lambda a: a.reshape(S, D).T
        out = call(A_shift_k.T, A_ssm_D, B_b1, B_b2, jnp.asarray(wf, bf16), jnp.asarray(wi, bf16),
                   tr(A_q), tr(A_k), tr(A_v), A_ssm_k, B_w1, B_w2)
        return out.T.reshape(1, S, D)
    return fn


_FN = _build()


def pallas_recurrent_scan__ssm_conv_h3__mixer_token_mlp__prompt_kernel(
        A_q, A_k, A_v, A_shift_k, A_ssm_k, A_ssm_D, B_x, B_w1, B_b1, B_w2, B_b2):
    return _FN(A_q, A_k, A_v, A_shift_k, A_ssm_k, A_ssm_D, B_x, B_w1, B_b1, B_w2, B_b2)
```

```python
import functools
import numpy as np
import jax
import jax.numpy as jnp
from jax import lax
from jax.experimental import pallas as pl
from jax.experimental.pallas import tpu as pltpu

S, D, F, KS = 2048, 576, 4608, 4
C = 128
NCH = S // C
TF = 512
N1 = F // TF
TS = 256
N2 = S // TS
KG = 512
EPS = 1e-5
bf16, f32, i32, u32 = jnp.bfloat16, jnp.float32, jnp.int32, jnp.uint32
DH = D // 2


def _dft_mats():
    t = np.arange(C, dtype=np.float64)[:, None]
    f = np.arange(C, dtype=np.float64)[None, :]
    w = np.exp(-1j * np.pi * (2 * f + 1) * t / (2 * C))
    phi = 1j * (1 - 2 * (np.arange(C) % 2))
    fwd, inv = [], []
    for r in range(4):
        wf = w * phi[None, :] ** (-r)
        fwd.append(np.concatenate([wf.real, wf.imag], axis=1))
        wi = np.conj(w).T * (phi ** r)[:, None] / C
        inv.append(np.concatenate([wi.real, -wi.imag], axis=0))
    return np.stack(fwd).astype(np.float32), np.stack(inv).astype(np.float32)


def _gelu(u):
    return 0.5 * u * (1.0 + jnp.tanh(0.7978845608028654 * (u + 0.044715 * (u * u * u))))


def pk(x):
    return pltpu.bitcast(x.astype(bf16), u32)


def unpk(x):
    return pltpu.bitcast(x, bf16)


def pin_f32(x, t):
    if t is None:
        return x
    tt = jnp.tile(t, (x.shape[0] // 8, x.shape[1] // 128))
    return pltpu.bitcast(pltpu.bitcast(x, i32) | tt, f32)


def _build(zg=2, zrows=144, nb=4, pin_every=1, wts=(3, 3, 3, 1), flags=None, sc_rows=16):
    ZS = zrows // 16

    def kern(sk_hbm, sd_hbm, b1_hbm, b2_hbm, wf_hbm, wi_hbm,
             x_hbm, k_hbm, v_hbm, ssm_hbm, w1_hbm, w2_hbm, o_hbm,
             sk_v, sd_v, b1r_v, b2r_v, wf_v, wi_v,
             x_v, k_v, v_v, ssm_v, w1_v, w2_v, o_v,
             xn_v, h_v, u_v, kv_v, kf_v, xf_v, z_v, b1_v, b2_v, skc_v, dc_v, y_v, yc_v, zero_v,
             sem_p, sem_w0, sem_x, sem_kv, sem_w1, sem_w2, sem_o):
        acp = pltpu.make_async_copy
        HS = S // 2
        def cx(p): return acp(x_hbm.at[:, pl.ds(p * TS, TS)], x_v.at[p], sem_x.at[p % 4])
        def ck(a): return acp(k_hbm.at[:, pl.ds(a * HS, HS)], k_v.at[a, :, pl.ds(C, HS)], sem_kv.at[a])
        def cv(a): return acp(v_hbm.at[:, pl.ds(a * HS, HS)], v_v.at[a], sem_kv.at[a])
        ckh = acp(k_hbm.at[:, pl.ds(HS - C, C)], k_v.at[1, :, pl.ds(0, C)], sem_kv.at[1])
        def cs(a): return acp(ssm_hbm.at[:, pl.ds(a * HS, HS)], ssm_v.at[:, pl.ds(a * HS, HS)], sem_p.at[2])
        def c1(j): return acp(w1_hbm.at[:, pl.ds(pl.multiple_of(j * TF, TF), TF)], w1_v.at[j], sem_w1.at[j % 2])
        def c2(i): return acp(w2_hbm.at[:, pl.ds(pl.multiple_of(i * TS, TS), TS)], w2_v.at[i], sem_w2.at[i % 3])
        def co(c): return acp(o_v.at[c], o_hbm.at[:, pl.ds(pl.multiple_of(c * C, C), C)], sem_o.at[0])
        small = [acp(s, d_, sem_p.at[min(n, 1)]) for n, (s, d_) in enumerate(
            [(b1_hbm, b1r_v), (b2_hbm, b2r_v), (sk_hbm, sk_v), (sd_hbm, sd_v), (wf_hbm, wf_v), (wi_hbm, wi_v)])]

        def c1p(kg): return acp(w1_hbm.at[pl.ds(kg * KG, KG), pl.ds(0, TF)], w1_v.at[0, pl.ds(kg * KG, KG), :], sem_w0.at[kg % 2])
        cx(0).start(); cx(1).start(); c1p(0).start()
        cx(2).start(); cx(3).start(); c1p(1).start()
        small[0].start()
        zero_v[...] = jnp.zeros((8, C), i32)

        def ln_steps(p):
            A, B, Cc = [], [], []
            for e in range(TS // C):
                ls = slice(e * C, (e + 1) * C)
                st_ = {}
                nrb = D // 16
                for rb in range(nrb):
                    rs = slice(16 * rb, 16 * rb + 16)
                    def sa(pin, rs=rs, rb=rb, ls=ls, st_=st_):
                        xf = pin_f32(x_v[p, rs, ls].astype(f32), None if pin is None else pin())
                        st_["a"] = xf if rb == 0 else st_["a"] + xf
                        if rb == nrb - 1:
                            st_["m"] = jnp.sum(st_["a"], axis=0, keepdims=True) * (1.0 / D)
                    def sb(pin, rs=rs, rb=rb, ls=ls, st_=st_):
                        d = pin_f32(x_v[p, rs, ls].astype(f32), None if pin is None else pin()) - st_["m"]
                        xn_v[p, rs, ls] = d
                        st_["s1"] = d if rb == 0 else st_["s1"] + d
                        st_["s2"] = d * d if rb == 0 else st_["s2"] + d * d
                        if rb == nrb - 1:
                            e_ = jnp.sum(st_["s1"], axis=0, keepdims=True) * (1.0 / D)
                            v = jnp.sum(st_["s2"], axis=0, keepdims=True) * (1.0 / D)
                            r = lax.rsqrt(v + EPS)
                            r2 = lax.rsqrt(r * r * (v - e_ * e_) + EPS)
                            st_["e"], st_["r"], st_["rr"] = e_, r, r * r2
                    def sc_(pin, rs=rs, rb=rb, ls=ls, e=e, st_=st_):
                        d = pin_f32(xn_v[p, rs, ls], None if pin is None else pin())
                        xn_v[p, rs, ls] = d * st_["r"]
                        h_v[8 * rb:8 * rb + 8, p * TS + e * C:p * TS + (e + 1) * C] = pk((d - st_["e"]) * st_["rr"])
                    A.append(sa); B.append(sb); Cc.append(sc_)
            mix = lambda L: [x for pair in zip(L[:len(L) // 2], L[len(L) // 2:]) for x in pair]
            return mix(A), mix(B), mix(Cc)

        def prep_steps():
            out = []
            def fill(pin):
                k_v[0, :, 0:C] = jnp.zeros((D, C), bf16)
                y_v[1] = jnp.zeros((D, C), f32)
                yc_v[1] = jnp.zeros((D, C), f32)
                b2r = b2r_v[...].astype(f32)[None, :]
                for i in range(N2):
                    b2_v[i] = b2r[:, i * TS:(i + 1) * TS]
            out.append(fill)
            for t in range(KS + 1):
                for c0 in range(0, D, C):
                    w = min(C, D - c0)
                    def st(pin, t=t, c0=c0, w=w):
                        row = sk_v[t:t + 1, c0:c0 + w].astype(f32) if t < KS else sd_v[...].astype(f32)[None, c0:c0 + w]
                        tile = jnp.broadcast_to(row, (C, w))
                        if w == C:
                            tile = pin_f32(tile, pin())
                        if t < KS:
                            skc_v[t, c0:c0 + w, :] = tile.T
                        else:
                            dc_v[c0:c0 + w, :] = tile.T
                    out.append(st)
            return out

        for p in range(2):
            cx(p).wait()
            for L in ln_steps(p):
                for st in L:
                    st(None)

        def run_pinned(y, steps):
            n = len(steps)
            z0 = zero_v[...]
            nv = y.shape[0] // 8
            for q, st in enumerate(steps):
                s = min(nv - 1, (q * nv) // n)
                st(lambda s=s: pltpu.bitcast(y[8 * s:8 * s + 8, 0:C], i32) & z0)

        def share(steps, weights):
            tot = sum(weights); out = []; lo = 0; acc = 0
            for w in weights:
                acc += w
                hi = (len(steps) * acc) // tot
                out.append(steps[lo:hi]); lo = hi
            return out

        def mlp1(j, steps=(), seg_w=None, after=None):
            segs = [(n, kg) for n in range(TF // C) for kg in range(S // KG)]
            w = seg_w if seg_w is not None else [wts[kg] for (n, kg) in segs]
            sh = share(list(steps), w)
            acc = None
            for q, (n, kg) in enumerate(segs):
                lhs = unpk(h_v[:, kg * KG:(kg + 1) * KG])
                y = jnp.dot(lhs, w1_v[j, kg * KG:(kg + 1) * KG, n * C:(n + 1) * C], preferred_element_type=f32)
                acc = y + b1_v[j, :, n * C:(n + 1) * C] if kg == 0 else acc + y
                if kg == S // KG - 1:
                    u_v[j, :, n * C:(n + 1) * C] = pk(_gelu(acc))
                run_pinned(y, sh[q])
                if after is not None:
                    after(q)

        accs = [None] * 4
        for kg in range(4):
            if kg + 2 < 4:
                cx(2 * kg + 4).start(); cx(2 * kg + 5).start()
            elif kg == 2:
                c1(1).start()
            else:
                for cp in small[1:]:
                    cp.start()
            if kg < 3:
                cx(2 * kg + 2).wait(); cx(2 * kg + 3).wait()
                A0, B0, C0 = ln_steps(2 * kg + 2)
                A1, B1, C1 = ln_steps(2 * kg + 3)
                zz = lambda a, b: [x for pair in zip(a, b) for x in pair]
                work = [zz(A0, A1), zz(B0, B1), zz(C0, C1), []]
            else:
                work = [[], [], [], []]
            c1p(kg).wait()
            if kg + 2 < 4:
                c1p(kg + 2).start()
            if kg == 3:
                small[0].wait()
                b1r = b1r_v[...].astype(f32)[None, :]
                for j in range(N1):
                    b1_v[j] = b1r[:, j * TF:(j + 1) * TF]
            for n in range(4):
                y = jnp.dot(unpk(h_v[:, kg * KG:(kg + 1) * KG]), w1_v[0, kg * KG:(kg + 1) * KG, n * C:(n + 1) * C],
                            preferred_element_type=f32)
                accs[n] = y if kg == 0 else accs[n] + y
                if kg == 3:
                    u_v[0, :, n * C:(n + 1) * C] = pk(_gelu(accs[n] + b1_v[0, :, n * C:(n + 1) * C]))
                run_pinned(y, work[n])

        def sc_steps(a):
            out = []
            for r0 in range(0, D, sc_rows):
                def st(pin, r0=r0):
                    rs = slice(r0, r0 + sc_rows)
                    kk = pin_f32(k_v[a, rs, :].astype(f32), pin())
                    ks = kk[:, C:] * jnp.tile(skc_v[0, rs, :], (1, HS // C))
                    for t in range(1, KS):
                        ks = ks + kk[:, C - t:C - t + HS] * jnp.tile(skc_v[t, rs, :], (1, HS // C))
                    vv = v_v[a, rs, :].astype(f32)
                    kv_v[a, r0 // 2:(r0 + sc_rows) // 2, :] = pk(ks * vv)
                out.append(st)
            return out

        def xdft(a, e):
            xf_v[a * 8 + e] = jnp.dot(unpk(kv_v[a, :, e * C:(e + 1) * C]), wf_v[e % 4], preferred_element_type=f32)

        def kdft(c):
            kf = jnp.dot(ssm_v[:, c * C:(c + 1) * C], wf_v[c % 4], preferred_element_type=f32)
            if c == 0:
                kf_v[c, :, :C] = kf[:, :C] + dc_v[...]
                kf_v[c, :, C:] = kf[:, C:]
            else:
                kf_v[c] = kf

        c1(2).start(); ck(0).start(); cv(0).start()
        c1(1).wait()
        for cp in small[1:]:
            cp.wait()
        mlp1(1, prep_steps(), seg_w=[1] * 16)

        def a_body(a, _):
            j = 2 + a
            @pl.when(a == 0)
            def _(): c1(3).start(); ck(1).start(); cv(1).start(); ckh.start()
            @pl.when(a == 1)
            def _(): c1(4).start(); cs(0).start(); cs(1).start()
            c1(j).wait(); ck(a).wait(); cv(a).wait()
            @pl.when(a == 1)
            def _(): ckh.wait()
            mlp1(j, sc_steps(a), seg_w=[1] * 8 + [0] * 8,
                 after=lambda q: xdft(a, q - 8) if q >= 8 else None)
            return 0
        lax.fori_loop(0, 2, a_body, 0)

        c1(5).start()
        c1(4).wait(); cs(0).wait(); cs(1).wait()
        mlp1(4, after=lambda q: kdft(q))

        def z_steps(r0):
            rows = pl.ds(pl.multiple_of(r0, 16), 16)
            rowsh = pl.ds(pl.multiple_of(r0 // 2, 8), 8)
            st_ = {"prev": None}
            out = []
            for i0 in range(0, NCH, zg):
                kc, acc = {}, {}
                for j in range(i0 + zg):
                    def st(pin, i0=i0, j=j, kc=kc, acc=acc):
                        xr, xi = xf_v[j, rows, :C], xf_v[j, rows, C:]
                        if j % pin_every == 0:
                            xr = pin_f32(xr, pin())
                        for i in range(max(i0, j), i0 + zg):
                            m = i - j
                            if m not in kc:
                                kc[m] = (kf_v[m, rows, :C], kf_v[m, rows, C:])
                            kr, ki = kc[m]
                            tr = xr * kr - xi * ki
                            ti = xr * ki + xi * kr
                            acc[i] = (tr, ti) if i not in acc else (acc[i][0] + tr, acc[i][1] + ti)
                        if j == i0 + zg - 1:
                            for i in range(i0, i0 + zg):
                                zr_, zi_ = acc[i]
                                if st_["prev"] is not None:
                                    zr_, zi_ = zr_ + st_["prev"][0], zi_ + st_["prev"][1]
                                st_["prev"] = acc[i]
                                z_v[i, rowsh, :C] = pk(zr_)
                                z_v[i, rowsh, C:] = pk(zi_)
                    out.append(st)
            return out

        def b_body(b, _):
            j = 5 + b
            @pl.when(j + 1 < N1)
            def _(): c1(j + 1).start()
            @pl.when(j >= N1 - 2)
            def _(): c2(j - (N1 - 2)).start()
            c1(j).wait()
            r0 = jnp.minimum(b * zrows, D - zrows)
            steps = []
            for e in range(ZS):
                steps += z_steps(r0 + e * 16)
            mlp1(j, steps)
            return 0
        lax.fori_loop(0, nb, b_body, 0)

        def ep_steps(slot, p, e, c):
            out = []
            for r0 in range(0, D, 16):
                def st(pin, r0=r0):
                    rs = slice(r0, r0 + 16)
                    y = pin_f32(y_v[slot, rs, :], None if pin is None else pin())
                    g = y * jax.nn.sigmoid(y)
                    o = x_v[p, rs, e * C:(e + 1) * C].astype(f32) + xn_v[p, rs, e * C:(e + 1) * C] * yc_v[slot, rs, :] * g
                    o_v[c, rs, :] = o.astype(bf16)
                out.append(st)
            return out

        def mlp2_chunk(i, e, steps, slot):
            sh = share(steps, [1] * N1)
            acc = None
            for kg in range(N1):
                y = jnp.dot(unpk(u_v[kg]), w2_v[i, kg * KG:(kg + 1) * KG, e * C:(e + 1) * C], preferred_element_type=f32)
                acc = y + b2_v[i, :, e * C:(e + 1) * C] if kg == 0 else acc + y
                run_pinned(y, sh[kg])
                if kg == 1:
                    c = 2 * i + e
                    yc_v[slot] = jnp.dot(unpk(z_v[c]), wi_v[c % 4], preferred_element_type=f32)
            y_v[slot] = acc

        def p2_body(i, _):
            @pl.when(i + 2 < N2)
            def _(): c2(i + 2).start()
            c2(i).wait()
            ip = jnp.maximum(i - 1, 0)
            prev_slot = jnp.where(i == 0, 1, 3)
            prev_c = jnp.where(i == 0, NCH, 2 * i - 1)
            mlp2_chunk(i, 0, ep_steps(prev_slot, ip, 1, prev_c), 2)
            @pl.when(i > 0)
            def _(): co(2 * i - 1).start()
            mlp2_chunk(i, 1, ep_steps(2, i, 0, 2 * i), 3)
            co(2 * i).start()
            return 0
        lax.fori_loop(0, N2, p2_body, 0)
        for st in ep_steps(3, N2 - 1, 1, NCH - 1):
            st(None)
        co(NCH - 1).start()
        for c in range(NCH):
            co(c).wait()

    hb = pl.BlockSpec(memory_space=pl.ANY)
    V = pltpu.VMEM
    dma = pltpu.SemaphoreType.DMA
    call = pl.pallas_call(
        kern,
        out_shape=jax.ShapeDtypeStruct((D, S), bf16),
        in_specs=[hb] * 12,
        out_specs=hb,
        scratch_shapes=[
            V((KS, D), bf16), V((D,), bf16), V((F,), bf16), V((S,), bf16), V((4, C, 2 * C), bf16), V((4, 2 * C, C), bf16),
            V((N2, D, TS), bf16), V((2, D, C + S // 2), bf16), V((2, D, S // 2), bf16), V((D, S), bf16),
            V((N1, S, TF), bf16), V((N2, F, TS), bf16), V((NCH + 1, D, C), bf16),
            V((N2, D, TS), f32), V((DH, S), u32), V((N1, DH, TF), u32), V((2, DH, S // 2), u32),
            V((NCH, D, 2 * C), f32), V((NCH, D, 2 * C), f32), V((NCH, DH, 2 * C), u32),
            V((N1, 1, TF), f32), V((N2, 1, TS), f32), V((KS, D, C), f32), V((D, C), f32),
            V((4, D, C), f32), V((4, D, C), f32), V((8, C), i32),
            dma((3,)), dma((2,)), dma((4,)), dma((2,)), dma((2,)), dma((3,)), dma((1,)),
        ],
        compiler_params=pltpu.CompilerParams(vmem_limit_bytes=120 * 2**20, flags=flags),
    )
    wf, wi = _dft_mats()

    @jax.jit
    def fn(A_q, A_k, A_v, A_shift_k, A_ssm_k, A_ssm_D, B_x, B_w1, B_b1, B_w2, B_b2):
        tr = lambda a: a.reshape(S, D).T
        out = call(A_shift_k.T, A_ssm_D, B_b1, B_b2, jnp.asarray(wf, bf16), jnp.asarray(wi, bf16),
                   tr(A_q), tr(A_k), tr(A_v), A_ssm_k, B_w1, B_w2)
        return out.T.reshape(1, S, D)
    return fn


_FN = _build()


def pallas_recurrent_scan__ssm_conv_h3__mixer_token_mlp__prompt_kernel(
        A_q, A_k, A_v, A_shift_k, A_ssm_k, A_ssm_D, B_x, B_w1, B_b1, B_w2, B_b2):
    return _FN(A_q, A_k, A_v, A_shift_k, A_ssm_k, A_ssm_D, B_x, B_w1, B_b1, B_w2, B_b2)
```

```python
import functools
import numpy as np
import jax
import jax.numpy as jnp
from jax import lax
from jax.experimental import pallas as pl
from jax.experimental.pallas import tpu as pltpu

S, D, F, KS = 2048, 576, 4608, 4
C = 128
NCH = S // C
TF = 512
N1 = F // TF
TS = 256
N2 = S // TS
KG = 512
EPS = 1e-5
bf16, f32, i32, u32 = jnp.bfloat16, jnp.float32, jnp.int32, jnp.uint32
DH = D // 2


def _dft_mats():
    t = np.arange(C, dtype=np.float64)[:, None]
    f = np.arange(C, dtype=np.float64)[None, :]
    w = np.exp(-1j * np.pi * (2 * f + 1) * t / (2 * C))
    phi = 1j * (1 - 2 * (np.arange(C) % 2))
    fwd, inv = [], []
    for r in range(4):
        wf = w * phi[None, :] ** (-r)
        fwd.append(np.concatenate([wf.real, wf.imag], axis=1))
        wi = np.conj(w).T * (phi ** r)[:, None] / C
        inv.append(np.concatenate([wi.real, -wi.imag], axis=0))
    return np.stack(fwd).astype(np.float32), np.stack(inv).astype(np.float32)


def _gelu(u):
    return 0.5 * u * (1.0 + jnp.tanh(0.7978845608028654 * (u + 0.044715 * (u * u * u))))


def pk(x):
    return pltpu.bitcast(x.astype(bf16), u32)


def unpk(x):
    return pltpu.bitcast(x, bf16)


def pin_f32(x, t):
    if t is None:
        return x
    tt = jnp.tile(t, (x.shape[0] // 8, x.shape[1] // 128))
    return pltpu.bitcast(pltpu.bitcast(x, i32) | tt, f32)


def _build(lnbal=1, zg=2, zrows=144, nb=4, pin_every=1, wts=(3, 3, 3, 1), flags=None, sc_rows=16):
    ZS = zrows // 16

    def kern(sk_hbm, sd_hbm, b1_hbm, b2_hbm, wf_hbm, wi_hbm,
             x_hbm, k_hbm, v_hbm, ssm_hbm, w1_hbm, w2_hbm, o_hbm,
             sk_v, sd_v, b1r_v, b2r_v, wf_v, wi_v,
             x_v, k_v, v_v, ssm_v, w1_v, w2_v, o_v,
             xn_v, h_v, u_v, kv_v, kf_v, xf_v, z_v, b1_v, b2_v, skc_v, dc_v, y_v, yc_v, zero_v,
             sem_p, sem_w0, sem_x, sem_kv, sem_w1, sem_w2, sem_o):
        acp = pltpu.make_async_copy
        HS = S // 2
        def cx(p): return acp(x_hbm.at[:, pl.ds(p * TS, TS)], x_v.at[p], sem_x.at[p % 4])
        def ck(a): return acp(k_hbm.at[:, pl.ds(a * HS, HS)], k_v.at[a, :, pl.ds(C, HS)], sem_kv.at[a])
        def cv(a): return acp(v_hbm.at[:, pl.ds(a * HS, HS)], v_v.at[a], sem_kv.at[a])
        ckh = acp(k_hbm.at[:, pl.ds(HS - C, C)], k_v.at[1, :, pl.ds(0, C)], sem_kv.at[1])
        def cs(a): return acp(ssm_hbm.at[:, pl.ds(a * HS, HS)], ssm_v.at[:, pl.ds(a * HS, HS)], sem_p.at[2])
        def c1(j): return acp(w1_hbm.at[:, pl.ds(pl.multiple_of(j * TF, TF), TF)], w1_v.at[j], sem_w1.at[j % 2])
        def c2(i): return acp(w2_hbm.at[:, pl.ds(pl.multiple_of(i * TS, TS), TS)], w2_v.at[i], sem_w2.at[i % 3])
        def co(c): return acp(o_v.at[c], o_hbm.at[:, pl.ds(pl.multiple_of(c * C, C), C)], sem_o.at[0])
        small = [acp(s, d_, sem_p.at[min(n, 1)]) for n, (s, d_) in enumerate(
            [(b1_hbm, b1r_v), (b2_hbm, b2r_v), (sk_hbm, sk_v), (sd_hbm, sd_v), (wf_hbm, wf_v), (wi_hbm, wi_v)])]

        def c1p(kg): return acp(w1_hbm.at[pl.ds(kg * KG, KG), pl.ds(0, TF)], w1_v.at[0, pl.ds(kg * KG, KG), :], sem_w0.at[kg % 2])
        cx(0).start(); cx(1).start(); c1p(0).start()
        cx(2).start(); cx(3).start(); c1p(1).start()
        small[0].start()
        zero_v[...] = jnp.zeros((8, C), i32)

        def ln_steps(p):
            A, B, Cc = [], [], []
            for e in range(TS // C):
                ls = slice(e * C, (e + 1) * C)
                st_ = {}
                nrb = D // 16
                for rb in range(nrb):
                    rs = slice(16 * rb, 16 * rb + 16)
                    def sa(pin, rs=rs, rb=rb, ls=ls, st_=st_):
                        xf = pin_f32(x_v[p, rs, ls].astype(f32), None if pin is None else pin())
                        st_["a"] = xf if rb == 0 else st_["a"] + xf
                        if rb == nrb - 1:
                            st_["m"] = jnp.sum(st_["a"], axis=0, keepdims=True) * (1.0 / D)
                    def sb(pin, rs=rs, rb=rb, ls=ls, st_=st_):
                        d = pin_f32(x_v[p, rs, ls].astype(f32), None if pin is None else pin()) - st_["m"]
                        xn_v[p, rs, ls] = d
                        st_["s1"] = d if rb == 0 else st_["s1"] + d
                        st_["s2"] = d * d if rb == 0 else st_["s2"] + d * d
                        if rb == nrb - 1:
                            e_ = jnp.sum(st_["s1"], axis=0, keepdims=True) * (1.0 / D)
                            v = jnp.sum(st_["s2"], axis=0, keepdims=True) * (1.0 / D)
                            r = lax.rsqrt(v + EPS)
                            r2 = lax.rsqrt(r * r * (v - e_ * e_) + EPS)
                            st_["e"], st_["r"], st_["rr"] = e_, r, r * r2
                    def sc_(pin, rs=rs, rb=rb, ls=ls, e=e, st_=st_):
                        d = pin_f32(xn_v[p, rs, ls], None if pin is None else pin())
                        xn_v[p, rs, ls] = d * st_["r"]
                        h_v[8 * rb:8 * rb + 8, p * TS + e * C:p * TS + (e + 1) * C] = pk((d - st_["e"]) * st_["rr"])
                    A.append(sa); B.append(sb); Cc.append(sc_)
            mix = lambda L: [x for pair in zip(L[:len(L) // 2], L[len(L) // 2:]) for x in pair]
            return mix(A), mix(B), mix(Cc)

        def prep_steps():
            out = []
            def fill(pin):
                k_v[0, :, 0:C] = jnp.zeros((D, C), bf16)
                y_v[1] = jnp.zeros((D, C), f32)
                yc_v[1] = jnp.zeros((D, C), f32)
                b2r = b2r_v[...].astype(f32)[None, :]
                for i in range(N2):
                    b2_v[i] = b2r[:, i * TS:(i + 1) * TS]
            out.append(fill)
            for t in range(KS + 1):
                for c0 in range(0, D, C):
                    w = min(C, D - c0)
                    def st(pin, t=t, c0=c0, w=w):
                        row = sk_v[t:t + 1, c0:c0 + w].astype(f32) if t < KS else sd_v[...].astype(f32)[None, c0:c0 + w]
                        tile = jnp.broadcast_to(row, (C, w))
                        if w == C:
                            tile = pin_f32(tile, pin())
                        if t < KS:
                            skc_v[t, c0:c0 + w, :] = tile.T
                        else:
                            dc_v[c0:c0 + w, :] = tile.T
                    out.append(st)
            return out

        for p in range(2):
            cx(p).wait()
            for L in ln_steps(p):
                for st in L:
                    st(None)

        def run_pinned(y, steps):
            n = len(steps)
            z0 = zero_v[...]
            nv = y.shape[0] // 8
            for q, st in enumerate(steps):
                s = min(nv - 1, (q * nv) // n)
                st(lambda s=s: pltpu.bitcast(y[8 * s:8 * s + 8, 0:C], i32) & z0)

        def share(steps, weights):
            tot = sum(weights); out = []; lo = 0; acc = 0
            for w in weights:
                acc += w
                hi = (len(steps) * acc) // tot
                out.append(steps[lo:hi]); lo = hi
            return out

        def mlp1(j, steps=(), seg_w=None, after=None):
            segs = [(n, kg) for n in range(TF // C) for kg in range(S // KG)]
            w = seg_w if seg_w is not None else [wts[kg] for (n, kg) in segs]
            sh = share(list(steps), w)
            acc = None
            for q, (n, kg) in enumerate(segs):
                lhs = unpk(h_v[:, kg * KG:(kg + 1) * KG])
                y = jnp.dot(lhs, w1_v[j, kg * KG:(kg + 1) * KG, n * C:(n + 1) * C], preferred_element_type=f32)
                acc = y + b1_v[j, :, n * C:(n + 1) * C] if kg == 0 else acc + y
                if kg == S // KG - 1:
                    u_v[j, :, n * C:(n + 1) * C] = pk(_gelu(acc))
                run_pinned(y, sh[q])
                if after is not None:
                    after(q)

        accs = [None] * 4
        for kg in range(4):
            if kg + 2 < 4:
                cx(2 * kg + 4).start(); cx(2 * kg + 5).start()
            elif kg == 2:
                c1(1).start()
            else:
                for cp in small[1:]:
                    cp.start()
            if kg < 3:
                cx(2 * kg + 2).wait(); cx(2 * kg + 3).wait()
                A0, B0, C0 = ln_steps(2 * kg + 2)
                A1, B1, C1 = ln_steps(2 * kg + 3)
                zz = lambda a, b: [x for pair in zip(a, b) for x in pair]
                work = [zz(A0, A1), zz(B0, B1), zz(C0, C1), []]
                if lnbal:
                    un = lambda L: (L[0::2], L[1::2])
                    (Bq0, Bq1), (Bq2, Bq3) = un(B0), un(B1)
                    (Cq0, Cq1), (Cq2, Cq3) = un(C0), un(C1)
                    z3 = lambda *ls: [x for tup in zip(*ls) for x in tup]
                    if lnbal == 1:
                        work = [zz(A0, A1), z3(Bq0, Bq1, Bq2), z3(Bq3, Cq0, Cq1), z3(Cq2, Cq3)]
                    else:
                        work = [zz(A0, A1), z3(Bq0, Bq1), z3(Bq2, Bq3, Cq0), z3(Cq1, Cq2, Cq3)]
            else:
                work = [[], [], [], []]
            c1p(kg).wait()
            if kg + 2 < 4:
                c1p(kg + 2).start()
            if kg == 3:
                small[0].wait()
                b1r = b1r_v[...].astype(f32)[None, :]
                for j in range(N1):
                    b1_v[j] = b1r[:, j * TF:(j + 1) * TF]
            for n in range(4):
                y = jnp.dot(unpk(h_v[:, kg * KG:(kg + 1) * KG]), w1_v[0, kg * KG:(kg + 1) * KG, n * C:(n + 1) * C],
                            preferred_element_type=f32)
                accs[n] = y if kg == 0 else accs[n] + y
                if kg == 3:
                    u_v[0, :, n * C:(n + 1) * C] = pk(_gelu(accs[n] + b1_v[0, :, n * C:(n + 1) * C]))
                run_pinned(y, work[n])

        def sc_steps(a):
            out = []
            for r0 in range(0, D, sc_rows):
                def st(pin, r0=r0):
                    rs = slice(r0, r0 + sc_rows)
                    kk = pin_f32(k_v[a, rs, :].astype(f32), pin())
                    ks = kk[:, C:] * jnp.tile(skc_v[0, rs, :], (1, HS // C))
                    for t in range(1, KS):
                        ks = ks + kk[:, C - t:C - t + HS] * jnp.tile(skc_v[t, rs, :], (1, HS // C))
                    vv = v_v[a, rs, :].astype(f32)
                    kv_v[a, r0 // 2:(r0 + sc_rows) // 2, :] = pk(ks * vv)
                out.append(st)
            return out

        def xdft(a, e):
            xf_v[a * 8 + e] = jnp.dot(unpk(kv_v[a, :, e * C:(e + 1) * C]), wf_v[e % 4], preferred_element_type=f32)

        def kdft(c):
            kf = jnp.dot(ssm_v[:, c * C:(c + 1) * C], wf_v[c % 4], preferred_element_type=f32)
            if c == 0:
                kf_v[c, :, :C] = kf[:, :C] + dc_v[...]
                kf_v[c, :, C:] = kf[:, C:]
            else:
                kf_v[c] = kf

        c1(2).start(); ck(0).start(); cv(0).start()
        c1(1).wait()
        for cp in small[1:]:
            cp.wait()
        mlp1(1, prep_steps(), seg_w=[1] * 16)

        def a_body(a, _):
            j = 2 + a
            @pl.when(a == 0)
            def _(): c1(3).start(); ck(1).start(); cv(1).start(); ckh.start()
            @pl.when(a == 1)
            def _(): c1(4).start(); cs(0).start(); cs(1).start()
            c1(j).wait(); ck(a).wait(); cv(a).wait()
            @pl.when(a == 1)
            def _(): ckh.wait()
            mlp1(j, sc_steps(a), seg_w=[1] * 8 + [0] * 8,
                 after=lambda q: xdft(a, q - 8) if q >= 8 else None)
            return 0
        lax.fori_loop(0, 2, a_body, 0)

        c1(5).start()
        c1(4).wait(); cs(0).wait(); cs(1).wait()
        mlp1(4, after=lambda q: kdft(q))

        def z_steps(r0):
            rows = pl.ds(pl.multiple_of(r0, 16), 16)
            rowsh = pl.ds(pl.multiple_of(r0 // 2, 8), 8)
            st_ = {"prev": None}
            out = []
            for i0 in range(0, NCH, zg):
                kc, acc = {}, {}
                for j in range(i0 + zg):
                    def st(pin, i0=i0, j=j, kc=kc, acc=acc):
                        xr, xi = xf_v[j, rows, :C], xf_v[j, rows, C:]
                        if j % pin_every == 0:
                            xr = pin_f32(xr, pin())
                        for i in range(max(i0, j), i0 + zg):
                            m = i - j
                            if m not in kc:
                                kc[m] = (kf_v[m, rows, :C], kf_v[m, rows, C:])
                            kr, ki = kc[m]
                            tr = xr * kr - xi * ki
                            ti = xr * ki + xi * kr
                            acc[i] = (tr, ti) if i not in acc else (acc[i][0] + tr, acc[i][1] + ti)
                        if j == i0 + zg - 1:
                            for i in range(i0, i0 + zg):
                                zr_, zi_ = acc[i]
                                if st_["prev"] is not None:
                                    zr_, zi_ = zr_ + st_["prev"][0], zi_ + st_["prev"][1]
                                st_["prev"] = acc[i]
                                z_v[i, rowsh, :C] = pk(zr_)
                                z_v[i, rowsh, C:] = pk(zi_)
                    out.append(st)
            return out

        def b_body(b, _):
            j = 5 + b
            @pl.when(j + 1 < N1)
            def _(): c1(j + 1).start()
            @pl.when(j >= N1 - 2)
            def _(): c2(j - (N1 - 2)).start()
            c1(j).wait()
            r0 = jnp.minimum(b * zrows, D - zrows)
            steps = []
            for e in range(ZS):
                steps += z_steps(r0 + e * 16)
            mlp1(j, steps)
            return 0
        lax.fori_loop(0, nb, b_body, 0)

        def ep_steps(slot, p, e, c):
            out = []
            for r0 in range(0, D, 16):
                def st(pin, r0=r0):
                    rs = slice(r0, r0 + 16)
                    y = pin_f32(y_v[slot, rs, :], None if pin is None else pin())
                    g = y * jax.nn.sigmoid(y)
                    o = x_v[p, rs, e * C:(e + 1) * C].astype(f32) + xn_v[p, rs, e * C:(e + 1) * C] * yc_v[slot, rs, :] * g
                    o_v[c, rs, :] = o.astype(bf16)
                out.append(st)
            return out

        def mlp2_chunk(i, e, steps, slot):
            sh = share(steps, [1] * N1)
            acc = None
            for kg in range(N1):
                y = jnp.dot(unpk(u_v[kg]), w2_v[i, kg * KG:(kg + 1) * KG, e * C:(e + 1) * C], preferred_element_type=f32)
                acc = y + b2_v[i, :, e * C:(e + 1) * C] if kg == 0 else acc + y
                run_pinned(y, sh[kg])
                if kg == 1:
                    c = 2 * i + e
                    yc_v[slot] = jnp.dot(unpk(z_v[c]), wi_v[c % 4], preferred_element_type=f32)
            y_v[slot] = acc

        def p2_body(i, _):
            @pl.when(i + 2 < N2)
            def _(): c2(i + 2).start()
            c2(i).wait()
            ip = jnp.maximum(i - 1, 0)
            prev_slot = jnp.where(i == 0, 1, 3)
            prev_c = jnp.where(i == 0, NCH, 2 * i - 1)
            mlp2_chunk(i, 0, ep_steps(prev_slot, ip, 1, prev_c), 2)
            @pl.when(i > 0)
            def _(): co(2 * i - 1).start()
            mlp2_chunk(i, 1, ep_steps(2, i, 0, 2 * i), 3)
            co(2 * i).start()
            return 0
        lax.fori_loop(0, N2, p2_body, 0)
        for st in ep_steps(3, N2 - 1, 1, NCH - 1):
            st(None)
        co(NCH - 1).start()
        for c in range(NCH):
            co(c).wait()

    hb = pl.BlockSpec(memory_space=pl.ANY)
    V = pltpu.VMEM
    dma = pltpu.SemaphoreType.DMA
    call = pl.pallas_call(
        kern,
        out_shape=jax.ShapeDtypeStruct((D, S), bf16),
        in_specs=[hb] * 12,
        out_specs=hb,
        scratch_shapes=[
            V((KS, D), bf16), V((D,), bf16), V((F,), bf16), V((S,), bf16), V((4, C, 2 * C), bf16), V((4, 2 * C, C), bf16),
            V((N2, D, TS), bf16), V((2, D, C + S // 2), bf16), V((2, D, S // 2), bf16), V((D, S), bf16),
            V((N1, S, TF), bf16), V((N2, F, TS), bf16), V((NCH + 1, D, C), bf16),
            V((N2, D, TS), f32), V((DH, S), u32), V((N1, DH, TF), u32), V((2, DH, S // 2), u32),
            V((NCH, D, 2 * C), f32), V((NCH, D, 2 * C), f32), V((NCH, DH, 2 * C), u32),
            V((N1, 1, TF), f32), V((N2, 1, TS), f32), V((KS, D, C), f32), V((D, C), f32),
            V((4, D, C), f32), V((4, D, C), f32), V((8, C), i32),
            dma((3,)), dma((2,)), dma((4,)), dma((2,)), dma((2,)), dma((3,)), dma((1,)),
        ],
        compiler_params=pltpu.CompilerParams(vmem_limit_bytes=120 * 2**20, flags=flags),
    )
    wf, wi = _dft_mats()

    @jax.jit
    def fn(A_q, A_k, A_v, A_shift_k, A_ssm_k, A_ssm_D, B_x, B_w1, B_b1, B_w2, B_b2):
        tr = lambda a: a.reshape(S, D).T
        out = call(A_shift_k.T, A_ssm_D, B_b1, B_b2, jnp.asarray(wf, bf16), jnp.asarray(wi, bf16),
                   tr(A_q), tr(A_k), tr(A_v), A_ssm_k, B_w1, B_w2)
        return out.T.reshape(1, S, D)
    return fn


_FN = _build()


def pallas_recurrent_scan__ssm_conv_h3__mixer_token_mlp__prompt_kernel(
        A_q, A_k, A_v, A_shift_k, A_ssm_k, A_ssm_D, B_x, B_w1, B_b1, B_w2, B_b2):
    return _FN(A_q, A_k, A_v, A_shift_k, A_ssm_k, A_ssm_D, B_x, B_w1, B_b1, B_w2, B_b2)
```
